```python
import jax
import jax.numpy as jnp

def _softmax(x, axis=-1):
    return jax.nn.softmax(x, axis=axis)

def _gelu(x):
    return jax.nn.gelu(x, approximate=True)

def _silu(x):
    return jax.nn.silu(x)

def _sigmoid(x):
    return jax.nn.sigmoid(x)

def _layernorm(x, axis=-1, eps=1e-05):
    m = jnp.mean(x, axis=axis, keepdims=True)
    v = jnp.var(x, axis=axis, keepdims=True)
    return (x - m) / jnp.sqrt(v + eps)

def _scatter_add(tgt, idx, src, axis=0):
    return tgt.at[idx].add(src)

def _segment_sum(src, seg, n):
    return jax.ops.segment_sum(src, seg, n)

class _Rng:

    def __init__(self, key):
        self._k = key

    def _next(self):
        self._k, sub = jax.random.split(self._k)
        return sub

    def normal(self, shape):
        return jax.random.normal(self._next(), shape, dtype=jnp.bfloat16)

    def randint(self, lo, hi, shape):
        return jax.random.randint(self._next(), shape, lo, hi, dtype=jnp.int32)

    def uniform(self, shape, lo=0.0, hi=1.0):
        return jax.random.uniform(self._next(), shape, jnp.bfloat16, lo, hi)

    def permutation(self, n):
        return jax.random.permutation(self._next(), n)
kernel_name = 'interleave_layers__linear_kernel_hedgehog__memory_aug_recurrent_mem_tr__prompt'

def setup_inputs():
    _rng = _Rng(jax.random.key(int.from_bytes(__import__("os").urandom(4), "little")))
    _w = lambda a: (lambda t: t.astype(jnp.bfloat16) if jnp.issubdtype(t.dtype, jnp.floating) else t)(jnp.asarray(a))

    def _A_setup():
        B, S, D, H = (1, 2048, 640, 32)
        Dh = D // H
        return {'x': _w((lambda *s: _rng.normal(s) * 0.05)(B, S, D)), 'wqkv': _w((lambda *s: _rng.normal(s) * 0.05)(D, 3 * D)), 'w_phi': _w((lambda *s: _rng.normal(s) * 0.05)(H, Dh, Dh) * Dh ** (-0.5)), 'wo': _w((lambda *s: _rng.normal(s) * 0.05)(D, D))}
    _A_in = _A_setup()

    def _B_setup():
        B, S, Dm = (1, 2048, 640)
        H, Dh = (32, 192)
        M, seg = (8, 32)
        seg = min(seg, S)
        S = S // seg * seg
        return {'x': _w((lambda *s: _rng.normal(s) * 0.05)(B, S, Dm)), 'mem0': _w((lambda *s: _rng.normal(s) * 0.05)(B, M, Dm)), 'Wq': _w((lambda *s: _rng.normal(s) * 0.05)(Dm, H, Dh) * Dm ** (-0.5)), 'Wk': _w((lambda *s: _rng.normal(s) * 0.05)(Dm, H, Dh) * Dm ** (-0.5)), 'Wv': _w((lambda *s: _rng.normal(s) * 0.05)(Dm, H, Dh) * Dm ** (-0.5)), 'Wo': _w((lambda *s: _rng.normal(s) * 0.05)(H, Dh, Dm) * (H * Dh) ** (-0.5)), 'seg_len': seg}
    _B_in = _B_setup()
    return {'A_x': _A_in['x'], 'A_wqkv': _A_in['wqkv'], 'A_w_phi': _A_in['w_phi'], 'A_wo': _A_in['wo'], 'B_x': _B_in['x'], 'B_mem0': _B_in['mem0'], 'B_Wq': _B_in['Wq'], 'B_Wk': _B_in['Wk'], 'B_Wv': _B_in['Wv'], 'B_Wo': _B_in['Wo'], 'B_seg_len': _B_in['seg_len']}

def reference(A_x, A_wqkv, A_w_phi, A_wo, B_x, B_mem0, B_Wq, B_Wk, B_Wv, B_Wo, B_seg_len):

    def _A_ref(x, wqkv, w_phi, wo):
        B, S, D = x.shape
        H = 32
        Dh = D // H
        qkv = (lambda x, *d: x.transpose(*d))((x @ wqkv).reshape(B, S, 3, H, Dh), 2, 0, 3, 1, 4)
        q, k, v = (qkv[0], qkv[1], qkv[2])
        pq = jnp.einsum('bhsd,hdf->bhsf', q, w_phi)
        pk = jnp.einsum('bhsd,hdf->bhsf', k, w_phi)
        phi_q = jnp.concatenate([_softmax(pq, axis=-1), _softmax(-pq, axis=-1)], axis=-1)
        phi_k = jnp.concatenate([_softmax(pk, axis=-1), _softmax(-pk, axis=-1)], axis=-1)
        kv = jnp.einsum('bhsf,bhsd->bhfd', phi_k, v)
        z = jnp.einsum('bhsf->bhf', phi_k)
        num = jnp.einsum('bhqf,bhfd->bhqd', phi_q, kv)
        den = jnp.einsum('bhqf,bhf->bhq', phi_q, z)[..., None] + 1e-06
        o = num / den
        return (lambda x, *d: x.transpose(*d))(o, 0, 2, 1, 3).reshape(B, S, D) @ wo

    def _B_ref(x, mem0, Wq, Wk, Wv, Wo, seg_len):
        B, S, Dm = x.shape
        H, Dh = (Wq.shape[1], Wq.shape[2])
        M = mem0.shape[1]
        scale = Dh ** (-0.5)
        n_seg = S // seg_len
        L = M + seg_len
        idx = jnp.arange(L)
        mask = (idx[:, None] < M) | (idx[:, None] >= idx[None, :])
        mem = mem0
        outs = []
        for s in range(n_seg):
            xs = x[:, s * seg_len:(s + 1) * seg_len, :].copy()
            h = jnp.concatenate([mem, xs], axis=1)
            q = jnp.einsum('btd,dhe->bhte', h, Wq)
            k = jnp.einsum('btd,dhe->bhte', h, Wk)
            v = jnp.einsum('btd,dhe->bhte', h, Wv)
            scores = jnp.einsum('bhqe,bhke->bhqk', q, k) * scale
            scores = jnp.where(mask[None, None], scores, -1000000000.0)
            p = _softmax(scores, axis=-1)
            o = jnp.einsum('bhqk,bhke->bhqe', p, v)
            o = jnp.einsum('bhte,hed->btd', o, Wo)
            mem = o[:, :M, :].copy()
            outs.append(o[:, M:, :])
        return jnp.concatenate(outs, axis=1)
    x = A_x
    x = x + _A_ref(_layernorm(x, axis=-1), A_wqkv, A_w_phi, A_wo)
    x = x + _B_ref(_layernorm(x, axis=-1), B_mem0, B_Wq, B_Wk, B_Wv, B_Wo, B_seg_len)
    x = x + _A_ref(_layernorm(x, axis=-1), A_wqkv, A_w_phi, A_wo)
    x = x + _B_ref(_layernorm(x, axis=-1), B_mem0, B_Wq, B_Wk, B_Wv, B_Wo, B_seg_len)
    return x
```

```python
import functools

import jax
import jax.numpy as jnp
from jax import lax
import jax.experimental.pallas as pl
import jax.experimental.pallas.tpu as pltpu

F32 = jnp.float32
BF16 = jnp.bfloat16
HA = 32
TB = 256
LOOK = 1


def _nn(a, b):
    return lax.dot_general(a, b, (((1,), (0,)), ((), ())), preferred_element_type=F32)


def _nt(a, b):
    return lax.dot_general(a, b, (((1,), (1,)), ((), ())), preferred_element_type=F32)


def _tn(a, b):
    return lax.dot_general(a, b, (((0,), (0,)), ((), ())), preferred_element_type=F32)


def _ln(x):
    m = jnp.mean(x, axis=-1, keepdims=True)
    d = x - m
    v = jnp.mean(d * d, axis=-1, keepdims=True)
    return d * lax.rsqrt(v + 1e-5)


def _iota(shape, dim):
    return lax.broadcasted_iota(jnp.int32, shape, dim)


def _phi(p, nf):
    sl = [p[f * HA:(f + 1) * HA] for f in range(nf)]
    mx = functools.reduce(jnp.maximum, sl)
    mn = functools.reduce(jnp.minimum, sl)
    out = []
    for e in ([jnp.exp(s - mx) for s in sl], [jnp.exp(mn - s) for s in sl]):
        r = 1.0 / functools.reduce(jnp.add, e)
        out += [t * r for t in e]
    return out


def _kernel(x_ref, wqkv_ref, phi_ref, wo_ref, mem_ref, wq_h, wk_h, wv_h, wob_h, o_ref,
            xs, hs, stage, wb, wob, wqT, wkT, wv, wop, kv, kvT, zacc, sems, *, seg, dh):
    S, D = x_ref.shape
    nf = D // HA
    M = mem_ref.shape[0]
    L = M + seg
    PW = 2 * dh
    NP = wob.shape[0] // PW

    cps = [pltpu.make_async_copy(w, stage.at[i], sems.at[i]) for i, w in enumerate((wq_h, wk_h, wv_h))]
    cps.append(pltpu.make_async_copy(wob_h, wob, sems.at[3]))
    for c in cps:
        c.start()

    r, c = _iota((D, D), 0), _iota((D, D), 1)
    rh = (r * (65536 // nf + 1)) >> 16
    rd = r - rh * nf
    sel = (rd[:, :phi_ref.shape[0]] == c[:, :phi_ref.shape[0]]).astype(BF16)
    bdT = jnp.where(rh == c % HA, _nn(sel, phi_ref[...]), 0.0).astype(BF16)
    wqT[...] = _nn(wqkv_ref[:, :D], bdT).T.astype(BF16)
    wkT[...] = _nn(wqkv_ref[:, D:2 * D], bdT).T.astype(BF16)
    perm = jnp.where((rh == c % HA) & (rd == c // HA), 1.0, 0.0).astype(BF16)
    wv[...] = _nn(wqkv_ref[:, 2 * D:], perm).astype(BF16)
    wop[...] = _tn(perm, wo_ref[...]).astype(BF16)

    def layer_a(src):
        kv[...] = jnp.zeros_like(kv)
        zacc[...] = jnp.zeros_like(zacc)

        def p1(i, _):
            rows = pl.ds(pl.multiple_of(i * TB, TB), TB)
            xn = _ln(src[rows, :].astype(F32))
            hs[rows, :] = xn
            xn = xn.astype(BF16)
            ph = jnp.concatenate(_phi(_nt(wkT[...], xn), nf), axis=0)
            v = _nn(xn, wv[...]).astype(BF16)
            kv[...] += _nn(ph.astype(BF16), v)
            zacc[...] += functools.reduce(jnp.add, [ph[:, j:j + 128] for j in range(0, TB, 128)])
            return 0
        lax.fori_loop(0, S // TB, p1, 0)

        m = _iota(kv.shape, 0) % HA == _iota(kv.shape, 1) % HA
        kvT[...] = jnp.where(m, kv[...], 0.0).T.astype(BF16)
        zacc[...] = jnp.broadcast_to(jnp.sum(zacc[...], axis=1, keepdims=True), zacc.shape)

        def p2(i, _):
            rows = pl.ds(pl.multiple_of(i * TB, TB), TB)
            xn = hs[rows, :].astype(BF16)
            ph = _phi(_nt(wqT[...], xn), nf)
            den = functools.reduce(jnp.add, [
                p * jnp.concatenate([zacc[j * HA:(j + 1) * HA, :]] * (TB // 128), axis=1)
                for j, p in enumerate(ph)])
            inv = 1.0 / (den + 1e-6)
            num = _nn(kvT[...], jnp.concatenate(ph, axis=0).astype(BF16))
            o = num * jnp.concatenate([inv] * nf, axis=0)
            x = src[rows, :].astype(F32) + _nn(o.T.astype(BF16), wop[...])
            xs[rows, :] = x
            hs[rows, :] = _ln(x)
            return 0
        lax.fori_loop(0, S // TB, p2, 0)

    def layer_b(dst):
        def step(s, mem):
            rows = pl.ds(pl.multiple_of(s * seg, seg), seg)
            h = jnp.concatenate([mem, hs[rows, :]], axis=0)
            lo = _iota((L, PW), 1) < dh
            qi, ci = _iota((L, 2 * L), 0), _iota((L, 2 * L), 1)
            ha = ci < L
            vis = (qi < M) | (qi >= jnp.where(ha, ci, ci - L))

            def bd(t):
                return jnp.concatenate([jnp.where(lo, t, 0.0), jnp.where(lo, 0.0, t)], axis=0).astype(BF16)

            def proj(g):
                q = _nn(h, wb[0, g])
                k = _nn(h, wb[1, g])
                sc = _nt(q, bd(k))
                return sc, bd(_nn(h, wb[2, g]))

            def attn(sc, vbd):
                sc = jnp.where(vis, sc * dh ** -0.5, -1e9)
                ma = jnp.max(jnp.where(ha, sc, -jnp.inf), axis=1, keepdims=True)
                mb = jnp.max(jnp.where(ha, -jnp.inf, sc), axis=1, keepdims=True)
                e = jnp.exp(sc - jnp.where(ha, ma, mb))
                sa = jnp.sum(jnp.where(ha, e, 0.0), axis=1, keepdims=True)
                sb = jnp.sum(jnp.where(ha, 0.0, e), axis=1, keepdims=True)
                return _nn(e * jnp.where(ha, 1.0 / sa, 1.0 / sb), vbd)

            acc = None
            pr, ot = {}, {}
            for t in range(NP + 2 * LOOK):
                if t < NP:
                    pr[t] = proj(t)
                g = t - LOOK
                if 0 <= g < NP:
                    ot[g] = attn(*pr.pop(g))
                g = t - 2 * LOOK
                if 0 <= g < NP:
                    y = _nn(ot.pop(g), wob[g * PW:(g + 1) * PW, :])
                    acc = y if acc is None else acc + y
            dst[rows, :] = (xs[rows, :] + acc[M:]).astype(dst.dtype)
            return acc[:M]
        lax.fori_loop(0, S // seg, step, mem_ref[...].astype(F32))

    layer_a(x_ref)
    for i in range(3):
        cps[i].wait()

        def tr(g, _):
            wb[i, g] = stage[i, pl.ds(pl.multiple_of(g * PW, PW), PW), :].T
            return 0
        lax.fori_loop(0, NP, tr, 0)
    cps[3].wait()
    layer_b(xs)
    layer_a(xs)
    layer_b(o_ref)


@functools.partial(jax.jit, static_argnames=("B_seg_len",))
def pallas_interleave_layers__linear_kernel_hedgehog__memory_aug_recurrent_mem_tr__prompt_kernel(
    A_x, A_wqkv, A_w_phi, A_wo, B_x, B_mem0, B_Wq, B_Wk, B_Wv, B_Wo, B_seg_len,
):
    _, S, D = A_x.shape
    _, H, dh = B_Wq.shape
    nf = D // HA
    N = H * dh
    phi = jnp.pad(A_w_phi.transpose(1, 2, 0).reshape(nf, D), ((0, 128 - nf), (0, 0)))
    wt = [w.transpose(1, 2, 0).reshape(N, D) for w in (B_Wq, B_Wk, B_Wv)]
    vm = pl.BlockSpec(memory_space=pltpu.VMEM)
    hbm = pl.BlockSpec(memory_space=pl.ANY)
    out = pl.pallas_call(
        functools.partial(_kernel, seg=int(B_seg_len), dh=dh),
        out_shape=jax.ShapeDtypeStruct((S, D), A_x.dtype),
        in_specs=[vm] * 5 + [hbm] * 4,
        out_specs=vm,
        scratch_shapes=[
            pltpu.VMEM((S, D), F32), pltpu.VMEM((S, D), F32),
            pltpu.VMEM((3, N, D), BF16), pltpu.VMEM((3, H // 2, D, 2 * dh), BF16),
            pltpu.VMEM((N, D), BF16),
            pltpu.VMEM((D, D), BF16), pltpu.VMEM((D, D), BF16),
            pltpu.VMEM((D, D), BF16), pltpu.VMEM((D, D), BF16),
            pltpu.VMEM((2 * D, D), F32), pltpu.VMEM((D, 2 * D), BF16),
            pltpu.VMEM((2 * D, 128), F32),
            pltpu.SemaphoreType.DMA((4,)),
        ],
        compiler_params=pltpu.CompilerParams(vmem_limit_bytes=110 * 1024 * 1024),
    )(A_x.reshape(S, D), A_wqkv, phi, A_wo, B_mem0[0], *wt, B_Wo.reshape(N, D))
    return out.reshape(A_x.shape)
```

```python
import functools

import jax
import jax.numpy as jnp
from jax import lax
import jax.experimental.pallas as pl
import jax.experimental.pallas.tpu as pltpu

F32 = jnp.float32
BF16 = jnp.bfloat16
HA = 32
TB = 512
LOOK = 1


def _nn(a, b):
    return lax.dot_general(a, b, (((1,), (0,)), ((), ())), preferred_element_type=F32)


def _nt(a, b):
    return lax.dot_general(a, b, (((1,), (1,)), ((), ())), preferred_element_type=F32)


def _tn(a, b):
    return lax.dot_general(a, b, (((0,), (0,)), ((), ())), preferred_element_type=F32)


def _ln(x):
    m = jnp.mean(x, axis=-1, keepdims=True)
    d = x - m
    v = jnp.mean(d * d, axis=-1, keepdims=True)
    return d * lax.rsqrt(v + 1e-5)


def _iota(shape, dim):
    return lax.broadcasted_iota(jnp.int32, shape, dim)


def _phi(p, nf):
    sl = [p[f * HA:(f + 1) * HA] for f in range(nf)]
    mx = functools.reduce(jnp.maximum, sl)
    mn = functools.reduce(jnp.minimum, sl)
    out = []
    for e in ([jnp.exp(s - mx) for s in sl], [jnp.exp(mn - s) for s in sl]):
        r = 1.0 / functools.reduce(jnp.add, e)
        out += [t * r for t in e]
    return out


def _kernel(x_ref, wqkv_ref, phi_ref, wo_ref, mem_ref, wq_h, wk_h, wv_h, wob_h, o_ref,
            xs, hs, stage, wb, wob, wqT, wkT, wv, wop, kv, kvT, zacc, sems, *, seg, dh):
    S, D = x_ref.shape
    nf = D // HA
    M = mem_ref.shape[0]
    L = M + seg
    PW = 2 * dh
    NP = wob.shape[0] // PW

    cps = [pltpu.make_async_copy(w, stage.at[i], sems.at[i]) for i, w in enumerate((wq_h, wk_h, wv_h))]
    cps.append(pltpu.make_async_copy(wob_h, wob, sems.at[3]))
    for c in cps:
        c.start()

    r, c = _iota((D, D), 0), _iota((D, D), 1)
    rh = (r * (65536 // nf + 1)) >> 16
    rd = r - rh * nf
    sel = (rd[:, :phi_ref.shape[0]] == c[:, :phi_ref.shape[0]]).astype(BF16)
    bdT = jnp.where(rh == c % HA, _nn(sel, phi_ref[...]), 0.0).astype(BF16)
    wqT[...] = _nn(wqkv_ref[:, :D], bdT).T.astype(BF16)
    wkT[...] = _nn(wqkv_ref[:, D:2 * D], bdT).T.astype(BF16)
    perm = jnp.where((rh == c % HA) & (rd == c // HA), 1.0, 0.0).astype(BF16)
    wv[...] = _nn(wqkv_ref[:, 2 * D:], perm).astype(BF16)
    wop[...] = _tn(perm, wo_ref[...]).astype(BF16)

    def layer_a(src, first=False):
        kv[...] = jnp.zeros_like(kv)
        zacc[...] = jnp.zeros_like(zacc)

        def p1(i, _):
            rows = pl.ds(pl.multiple_of(i * TB, TB), TB)
            xn = _ln(src[rows, :].astype(F32))
            hs[rows, :] = xn
            xn = xn.astype(BF16)
            ph = jnp.concatenate(_phi(_nt(wkT[...], xn), nf), axis=0)
            v = _nn(xn, wv[...]).astype(BF16)
            kv[...] += _nn(ph.astype(BF16), v)
            zacc[...] += functools.reduce(jnp.add, [ph[:, j:j + 128] for j in range(0, TB, 128)])
            return 0
        lax.fori_loop(0, S // TB, p1, 0)

        m = _iota(kv.shape, 0) % HA == _iota(kv.shape, 1) % HA
        kvT[...] = jnp.where(m, kv[...], 0.0).T.astype(BF16)
        zacc[...] = jnp.broadcast_to(jnp.sum(zacc[...], axis=1, keepdims=True), zacc.shape)

        if first:
            for c in cps[:3]:
                c.wait()

        def p2(i, _):
            rows = pl.ds(pl.multiple_of(i * TB, TB), TB)
            xn = hs[rows, :].astype(BF16)
            ph = _phi(_nt(wqT[...], xn), nf)
            den = functools.reduce(jnp.add, [
                p * jnp.concatenate([zacc[j * HA:(j + 1) * HA, :]] * (TB // 128), axis=1)
                for j, p in enumerate(ph)])
            inv = 1.0 / (den + 1e-6)
            num = _nn(kvT[...], jnp.concatenate(ph, axis=0).astype(BF16))
            o = num * jnp.concatenate([inv] * nf, axis=0)
            x = src[rows, :].astype(F32) + _nn(o.T.astype(BF16), wop[...])
            xs[rows, :] = x
            hs[rows, :] = _ln(x)
            if first:
                n = NP // (S // TB)
                for w in range(3):
                    for j in range(n):
                        g = i * n + j
                        wb[w, g] = stage[w, pl.ds(pl.multiple_of(g * PW, PW), PW), :].T
            return 0
        lax.fori_loop(0, S // TB, p2, 0)

    def layer_b(dst):
        def step(s, mem):
            rows = pl.ds(pl.multiple_of(s * seg, seg), seg)
            h = jnp.concatenate([mem, hs[rows, :]], axis=0)
            lo = _iota((L, PW), 1) < dh
            qi, ci = _iota((L, 2 * L), 0), _iota((L, 2 * L), 1)
            ha = ci < L
            vis = (qi < M) | (qi >= jnp.where(ha, ci, ci - L))

            def bd(t):
                return jnp.concatenate([jnp.where(lo, t, 0.0), jnp.where(lo, 0.0, t)], axis=0).astype(BF16)

            def proj(g):
                q = _nn(h, wb[0, g])
                k = _nn(h, wb[1, g])
                sc = _nt(q, bd(k))
                return sc, bd(_nn(h, wb[2, g]))

            def attn(sc, vbd):
                sc = jnp.where(vis, sc * dh ** -0.5, -1e9)
                ma = jnp.max(jnp.where(ha, sc, -jnp.inf), axis=1, keepdims=True)
                mb = jnp.max(jnp.where(ha, -jnp.inf, sc), axis=1, keepdims=True)
                e = jnp.exp(sc - jnp.where(ha, ma, mb))
                sa = jnp.sum(jnp.where(ha, e, 0.0), axis=1, keepdims=True)
                sb = jnp.sum(jnp.where(ha, 0.0, e), axis=1, keepdims=True)
                return _nn(e, vbd) * jnp.where(lo, 1.0 / sa, 1.0 / sb)

            acc = None
            pr, ot = {}, {}
            for t in range(NP + 2 * LOOK):
                if t < NP:
                    pr[t] = proj(t)
                g = t - LOOK
                if 0 <= g < NP:
                    ot[g] = attn(*pr.pop(g))
                g = t - 2 * LOOK
                if 0 <= g < NP:
                    y = _nn(ot.pop(g), wob[g * PW:(g + 1) * PW, :])
                    acc = y if acc is None else acc + y
            dst[rows, :] = (xs[rows, :] + acc[M:]).astype(dst.dtype)
            return acc[:M]
        lax.fori_loop(0, S // seg, step, mem_ref[...].astype(F32))

    layer_a(x_ref, True)
    cps[3].wait()
    layer_b(xs)
    layer_a(xs)
    layer_b(o_ref)


@functools.partial(jax.jit, static_argnames=("B_seg_len",))
def pallas_interleave_layers__linear_kernel_hedgehog__memory_aug_recurrent_mem_tr__prompt_kernel(
    A_x, A_wqkv, A_w_phi, A_wo, B_x, B_mem0, B_Wq, B_Wk, B_Wv, B_Wo, B_seg_len,
):
    _, S, D = A_x.shape
    _, H, dh = B_Wq.shape
    nf = D // HA
    N = H * dh
    phi = jnp.pad(A_w_phi.transpose(1, 2, 0).reshape(nf, D), ((0, 128 - nf), (0, 0)))
    wt = [w.transpose(1, 2, 0).reshape(N, D) for w in (B_Wq, B_Wk, B_Wv)]
    vm = pl.BlockSpec(memory_space=pltpu.VMEM)
    hbm = pl.BlockSpec(memory_space=pl.ANY)
    out = pl.pallas_call(
        functools.partial(_kernel, seg=int(B_seg_len), dh=dh),
        out_shape=jax.ShapeDtypeStruct((S, D), A_x.dtype),
        in_specs=[vm] * 5 + [hbm] * 4,
        out_specs=vm,
        scratch_shapes=[
            pltpu.VMEM((S, D), F32), pltpu.VMEM((S, D), F32),
            pltpu.VMEM((3, N, D), BF16), pltpu.VMEM((3, H // 2, D, 2 * dh), BF16),
            pltpu.VMEM((N, D), BF16),
            pltpu.VMEM((D, D), BF16), pltpu.VMEM((D, D), BF16),
            pltpu.VMEM((D, D), BF16), pltpu.VMEM((D, D), BF16),
            pltpu.VMEM((2 * D, D), F32), pltpu.VMEM((D, 2 * D), BF16),
            pltpu.VMEM((2 * D, 128), F32),
            pltpu.SemaphoreType.DMA((4,)),
        ],
        compiler_params=pltpu.CompilerParams(vmem_limit_bytes=110 * 1024 * 1024),
    )(A_x.reshape(S, D), A_wqkv, phi, A_wo, B_mem0[0], *wt, B_Wo.reshape(N, D))
    return out.reshape(A_x.shape)
```
